```python
import jax
import jax.numpy as jnp

def _softmax(x, axis=-1):
    return jax.nn.softmax(x, axis=axis)
def _gelu(x):
    return jax.nn.gelu(x, approximate=True)
def _silu(x):
    return jax.nn.silu(x)
def _sigmoid(x):
    return jax.nn.sigmoid(x)
def _layernorm(x, axis=-1, eps=1e-5):
    m = jnp.mean(x, axis=axis, keepdims=True)
    v = jnp.var(x, axis=axis, keepdims=True)
    return (x - m) / jnp.sqrt(v + eps)
def _scatter_add(tgt, idx, src, axis=0):
    return tgt.at[idx].add(src)
def _segment_sum(src, seg, n):
    return jax.ops.segment_sum(src, seg, n)
class _Rng:
    def __init__(self, key):
        self._k = key
    def _next(self):
        self._k, sub = jax.random.split(self._k)
        return sub
    def normal(self, shape):
        return jax.random.normal(self._next(), shape, dtype=jnp.bfloat16)
    def randint(self, lo, hi, shape):
        return jax.random.randint(self._next(), shape, lo, hi, dtype=jnp.int32)
    def uniform(self, shape, lo=0.0, hi=1.0):
        return jax.random.uniform(self._next(), shape, jnp.bfloat16, lo, hi)
    def permutation(self, n):
        return jax.random.permutation(self._next(), n)


kernel_name = 'standalone__self_sup_conv_stem_wavlm__speech'

def setup_inputs():
    _rng = _Rng(jax.random.key(int.from_bytes(__import__("os").urandom(4), "little")))
    _w = (lambda a: (lambda t: t.astype(jnp.bfloat16) if jnp.issubdtype(t.dtype, jnp.floating) else t)(jnp.asarray(a)))
    B, T, D, K = 2, 16000, 512, 31
    scale = (K * D) ** -0.5
    return {
        "x": _w((lambda *s: _rng.normal(s) * 0.05)(B, T, D)),
        "w": _w((lambda *s: _rng.normal(s) * 0.05)(K, D, D) * scale),
        "gn_gamma": _w((lambda *s: _rng.normal(s) * 0.05)(D) * 0.1 + 1.0),
        "gn_beta": _w((lambda *s: _rng.normal(s) * 0.05)(D) * 0.1),
    }

def reference(x, w, gn_gamma, gn_beta):
    B, T, D = x.shape
    K = w.shape[0]
    s = 2
    L = (T - K) // s + 1
    h = jnp.einsum('blc,cd->bld', x[:, 0:s * L:s, :], w[0])
    for i in range(1, K):
        h = h + jnp.einsum('blc,cd->bld', x[:, i:i + s * L:s, :], w[i])
    mu = jnp.einsum('bld->bd', h)[:, None, :] / L
    var = jnp.einsum('bld->bd', (h - mu) ** 2)[:, None, :] / L
    h = (h - mu) / jnp.sqrt(var + 1e-5)
    h = h * gn_gamma[None, None, :] + gn_beta[None, None, :]
    return _gelu(h)
```

```python
import functools

import numpy as np
import jax
import jax.numpy as jnp
from jax import lax
import jax.experimental.pallas as pl
import jax.experimental.pallas.tpu as pltpu

N = 64
NF = N // 2
M_OUT = 48
NTAP = 16
OUT_ROWS = 512


def _constants():
    theta = 2.0 * np.pi * (np.arange(NF) + 0.5) / N
    t = np.arange(N)
    ang = theta[:, None] * t[None, :]
    fr = np.concatenate([np.cos(ang), -np.sin(ang)], axis=0)
    f2 = np.zeros((2, 2 * NF, N, 2), np.float32)
    for p in range(2):
        f2[p, :, :, p] = fr
    f2 = f2.reshape(4 * NF, 2 * N)
    j = np.arange(NTAP)
    ang = theta[:, None] * j[None, :]
    g = np.concatenate([np.cos(ang), np.sin(ang)], axis=0)
    g8 = np.kron(g, np.eye(8)).astype(np.float32)
    m = np.arange(M_OUT)
    ang = m[:, None] * theta[None, :]
    a = np.stack([np.cos(ang), -np.sin(ang)], axis=-1).reshape(M_OUT, N) * (2.0 / N)
    a2 = np.kron(np.eye(2), a).astype(np.float32)
    return f2, g8, a2


def _gelu(x):
    c = np.float32(np.sqrt(2.0 / np.pi))
    u = x * (c + (c * np.float32(0.044715)) * (x * x))
    hx = 0.5 * x
    return hx + hx * jnp.tanh(u)


def _kernel(x_hbm, w_hbm, gam_ref, bet_ref, f2_ref, g8_ref, a2_ref, o_ref,
            wt_ref, xbuf, hbuf, sc_ref, xsem, *, B, T, D, K, L, NB):
    b = pl.program_id(0)
    j = pl.program_id(1)
    NP = NB // 2
    CT = D // 128
    WPIECE = 64
    NWP = D // WPIECE

    def x_copy(bb):
        return pltpu.make_async_copy(x_hbm.at[bb], xbuf.at[pl.ds(0, T)], xsem.at[0])

    @pl.when((b == 0) & (j == 0))
    def _weights():
        def body(wraw, wsem):
            def w_copy(i):
                return pltpu.make_async_copy(
                    w_hbm.at[:, pl.ds(i * WPIECE, WPIECE), :],
                    wraw.at[:, pl.ds(i * WPIECE, WPIECE), :], wsem.at[i])
            for i in range(NWP):
                w_copy(i).start()
            x_copy(0).start()
            xbuf[pl.ds(T, xbuf.shape[0] - T), :] = jnp.zeros(
                (xbuf.shape[0] - T, D), xbuf.dtype)

            low = lax.broadcasted_iota(jnp.int32, (8, D), 0) < 4

            def group(G, _):
                r0 = pl.multiple_of(G * 16, 16)
                g8 = g8_ref[...]
                for p in range(2):
                    def tap(jj):
                        i = 2 * jj + p
                        if i >= K:
                            return jnp.zeros((8, D), jnp.uint32)
                        return pltpu.bitcast(wraw[i, pl.ds(r0, 16), :], jnp.uint32)
                    lo, hi = [], []
                    for jp in range(NTAP // 2):
                        ta, tb = tap(2 * jp), tap(2 * jp + 1)
                        lo.append(jnp.where(low, ta, pltpu.roll(tb, 4, 0)))
                        hi.append(jnp.where(low, pltpu.roll(ta, 4, 0), tb))
                    lo = pltpu.bitcast(jnp.concatenate(lo, axis=0), jnp.bfloat16)
                    hi = pltpu.bitcast(jnp.concatenate(hi, axis=0), jnp.bfloat16)
                    rl = jnp.dot(g8, lo, preferred_element_type=jnp.float32)
                    rh = jnp.dot(g8, hi, preferred_element_type=jnp.float32)
                    for ri in range(2):
                        for k in range(NF):
                            r = (ri * NF + k) * 8
                            v = jnp.concatenate([rl[r:r + 8], rh[r:r + 8]], axis=0)
                            wt_ref[k, pl.ds(p * D + r0, 16), ri * D:(ri + 1) * D] = (
                                v.astype(jnp.bfloat16))
                return 0

            def piece(i, _):
                w_copy(i).wait()
                lax.fori_loop(i * (WPIECE // 16), (i + 1) * (WPIECE // 16), group, 0)
                return 0
            lax.fori_loop(0, NWP, piece, 0)

        pl.run_scoped(body, pltpu.VMEM((K, D, D), jnp.bfloat16),
                      pltpu.SemaphoreType.DMA((NWP,)))

    @pl.when(j == 0)
    def _conv():
        def body(dbuf, ybuf):
            x_copy(b).wait()

            def fwd(q, _):
                f2 = f2_ref[...]
                r = pl.multiple_of(q * (4 * M_OUT), 16)
                x0 = xbuf[pl.ds(r, 2 * N), :]
                x1 = xbuf[pl.ds(r + 2 * M_OUT, 2 * N), :]
                r0 = jnp.dot(f2, x0, preferred_element_type=jnp.float32)
                r1 = jnp.dot(f2, x1, preferred_element_type=jnp.float32)
                pk = pltpu.pack_elementwise([r0, r1], packed_dtype=jnp.bfloat16)
                for p in range(2):
                    for ri in range(2):
                        rr = (p * 2 + ri) * NF
                        for ct in range(CT):
                            dbuf[p * CT + ct, pl.ds(ri * NP + q, NF, stride=NB), :] = (
                                pk[rr:rr + NF, ct * 128:(ct + 1) * 128])
                return 0
            lax.fori_loop(0, NP, fwd, 0)

            @pl.when(b + 1 < B)
            def _():
                x_copy(b + 1).start()

            def mix(k, _):
                r = pl.multiple_of(k * NB, 8)
                lhs = jnp.concatenate(
                    [dbuf[s, pl.ds(r, NB), :] for s in range(2 * CT)], axis=1)
                lhs = pltpu.bitcast(lhs, jnp.bfloat16)
                res = jnp.dot(lhs, wt_ref[k], preferred_element_type=jnp.float32)
                yr = res[:NB, :D] - res[NB:, D:]
                yi = res[:NB, D:] + res[NB:, :D]
                pk = pltpu.pack_elementwise([yr, yi], packed_dtype=jnp.bfloat16)
                for ct in range(CT):
                    ybuf[ct, pl.ds(r, NB), :] = pk[:, ct * 128:(ct + 1) * 128]
                return 0
            lax.fori_loop(0, NF, mix, 0)

            RP = 2 * M_OUT

            def inv(q):
                parts = []
                for s in range(2):
                    parts.append(jnp.concatenate(
                        [ybuf[ct, pl.ds(2 * q + s, NF, stride=NB), :] for ct in range(CT)],
                        axis=1))
                rhs = pltpu.bitcast(jnp.concatenate(parts, axis=0), jnp.bfloat16)
                return jnp.dot(a2_ref[...], rhs, preferred_element_type=jnp.float32)

            def fold(y):
                acc = y[0:8]
                for i in range(1, y.shape[0] // 8):
                    acc = acc + y[8 * i:8 * i + 8]
                return acc

            def inv_body(q, s1):
                y = inv(q)
                hbuf[pl.ds(pl.multiple_of(q * RP, 16), RP), :] = y.astype(hbuf.dtype)
                return s1 + fold(y)
            nfull = L // RP
            s1 = lax.fori_loop(0, nfull, inv_body, jnp.zeros((8, D), jnp.float32))
            for q in range(nfull, NP):
                y = inv(q)
                valid = lax.broadcasted_iota(jnp.int32, y.shape, 0) < (L - q * RP)
                y = jnp.where(valid, y, 0.0)
                hbuf[pl.ds(q * RP, RP), :] = y.astype(hbuf.dtype)
                s1 = s1 + fold(y)
            mu = jnp.sum(s1, axis=0, keepdims=True) * np.float32(1.0 / L)

            def var_body(q, s2):
                d = hbuf[pl.ds(pl.multiple_of(q * RP, 16), RP), :].astype(jnp.float32) - mu
                return s2 + fold(d * d)
            s2 = lax.fori_loop(0, nfull, var_body, jnp.zeros((8, D), jnp.float32))
            for q in range(nfull, NP):
                d = hbuf[pl.ds(q * RP, RP), :].astype(jnp.float32) - mu
                valid = lax.broadcasted_iota(jnp.int32, d.shape, 0) < (L - q * RP)
                s2 = s2 + fold(jnp.where(valid, d * d, 0.0))
            var = jnp.sum(s2, axis=0, keepdims=True) * np.float32(1.0 / L)
            scale = lax.rsqrt(var + np.float32(1e-5)) * gam_ref[...].astype(jnp.float32)
            sc_ref[0:1, :] = mu
            sc_ref[1:2, :] = scale
            sc_ref[2:3, :] = bet_ref[...].astype(jnp.float32)

        pl.run_scoped(body,
                      pltpu.VMEM((2 * CT, NF * NB, 128), jnp.uint32),
                      pltpu.VMEM((CT, NF * NB, 128), jnp.uint32))

    mu = sc_ref[0:1, :]
    scale = sc_ref[1:2, :]
    beta = sc_ref[2:3, :]
    CH = 64

    def norm(i, _):
        r = pl.multiple_of(i * CH, CH)
        h = hbuf[pl.ds(pl.multiple_of(j * OUT_ROWS, OUT_ROWS) + r, CH), :].astype(jnp.float32)
        o_ref[pl.ds(r, CH), :] = _gelu((h - mu) * scale + beta).astype(o_ref.dtype)
        return 0
    lax.fori_loop(0, OUT_ROWS // CH, norm, 0)


@jax.jit
def pallas_standalone__self_sup_conv_stem_wavlm__speech_kernel(
    x: jax.Array,
    w: jax.Array,
    gn_gamma: jax.Array,
    gn_beta: jax.Array,
):
    B, T, D = x.shape
    K = w.shape[0]
    L = (T - K) // 2 + 1
    assert (K + 1) // 2 <= NTAP and D % 128 == 0 and T % 16 == 0
    NB = -(-L // M_OUT)
    NB = -(-NB // 16) * 16 if (NB % 8) else NB
    NB += NB % 2
    NB = -(-L // (2 * M_OUT)) * 2
    NB = -(-NB // 8) * 8
    NJ = -(-L // OUT_ROWS)
    hrows = max(NB * M_OUT, NJ * OUT_ROWS)
    xrows = 2 * M_OUT * (NB - 1) + 2 * N
    xrows = max(xrows, T + 16)
    f2, g8, a2 = _constants()
    dt = x.dtype
    consts = [jnp.asarray(c, dtype=jnp.bfloat16) for c in (f2, g8, a2)]

    def full(shape):
        return pl.BlockSpec(shape, lambda b, j: (0,) * len(shape))

    kern = functools.partial(_kernel, B=B, T=T, D=D, K=K, L=L, NB=NB)
    return pl.pallas_call(
        kern,
        grid=(B, NJ),
        in_specs=[
            pl.BlockSpec(memory_space=pl.ANY),
            pl.BlockSpec(memory_space=pl.ANY),
            full((1, D)), full((1, D)),
            full(f2.shape), full(g8.shape), full(a2.shape),
        ],
        out_specs=pl.BlockSpec((None, OUT_ROWS, D), lambda b, j: (b, j, 0)),
        out_shape=jax.ShapeDtypeStruct((B, L, D), dt),
        scratch_shapes=[
            pltpu.VMEM((NF, 2 * D, 2 * D), jnp.bfloat16),
            pltpu.VMEM((xrows, D), jnp.bfloat16),
            pltpu.VMEM((hrows, D), jnp.bfloat16),
            pltpu.VMEM((8, D), jnp.float32),
            pltpu.SemaphoreType.DMA((1,)),
        ],
        compiler_params=pltpu.CompilerParams(
            dimension_semantics=("arbitrary", "arbitrary"),
            vmem_limit_bytes=126 * 1024 * 1024),
    )(x.astype(jnp.bfloat16), w.astype(jnp.bfloat16),
      gn_gamma.reshape(1, D), gn_beta.reshape(1, D), *consts)
```

```python
import functools

import numpy as np
import jax
import jax.numpy as jnp
from jax import lax
import jax.experimental.pallas as pl
import jax.experimental.pallas.tpu as pltpu

N = 64
NF = N // 2
M_OUT = 48
NTAP = 16
INV_UNROLL = 4
OUT_ROWS = 512


def _constants():
    theta = 2.0 * np.pi * (np.arange(NF) + 0.5) / N
    t = np.arange(N)
    ang = theta[:, None] * t[None, :]
    fr = np.concatenate([np.cos(ang), -np.sin(ang)], axis=0)
    f2 = np.zeros((2, 2 * NF, N, 2), np.float32)
    for p in range(2):
        f2[p, :, :, p] = fr
    f2 = f2.reshape(4 * NF, 2 * N)
    j = np.arange(NTAP)
    ang = theta[:, None] * j[None, :]
    g = np.concatenate([np.cos(ang), np.sin(ang)], axis=0)
    g8 = np.kron(g, np.eye(8)).astype(np.float32)
    m = np.arange(M_OUT)
    ang = m[:, None] * theta[None, :]
    a = np.stack([np.cos(ang), -np.sin(ang)], axis=-1).reshape(M_OUT, N) * (2.0 / N)
    a2 = np.kron(np.eye(2), a).astype(np.float32)
    return f2, g8, a2


def _gelu(x):
    c = np.float32(np.sqrt(2.0 / np.pi))
    u = x * (c + (c * np.float32(0.044715)) * (x * x))
    hx = 0.5 * x
    return hx + hx * jnp.tanh(u)


def _kernel(x_hbm, w_hbm, gam_ref, bet_ref, f2_ref, g8_ref, a2_ref, o_ref,
            wt_ref, xbuf, hbuf, sc_ref, xsem, *, B, T, D, K, L, NB):
    j = pl.program_id(0)
    NP = NB // 2
    CT = D // 128
    WPIECE = 64
    NWP = D // WPIECE
    RP = 2 * M_OUT
    nfull = L // RP
    hrefs = (hbuf, xbuf)

    def x_copy(bb):
        return pltpu.make_async_copy(x_hbm.at[bb], xbuf.at[pl.ds(0, T)], xsem.at[0])

    def weights(wraw, wsem):
        def w_copy(i):
            return pltpu.make_async_copy(
                w_hbm.at[:, pl.ds(i * WPIECE, WPIECE), :],
                wraw.at[:, pl.ds(i * WPIECE, WPIECE), :], wsem.at[i])
        for i in range(NWP):
            w_copy(i).start()
        x_copy(0).start()
        xbuf[pl.ds(T, xbuf.shape[0] - T), :] = jnp.zeros(
            (xbuf.shape[0] - T, D), xbuf.dtype)
        if hbuf.shape[0] > NB * M_OUT:
            hbuf[pl.ds(NB * M_OUT, hbuf.shape[0] - NB * M_OUT), :] = jnp.zeros(
                (hbuf.shape[0] - NB * M_OUT, D), hbuf.dtype)

        low = lax.broadcasted_iota(jnp.int32, (8, D), 0) < 4

        def group(G, _):
            r0 = pl.multiple_of(G * 16, 16)
            g8 = g8_ref[...]
            for p in range(2):
                def tap(jj):
                    i = 2 * jj + p
                    if i >= K:
                        return jnp.zeros((8, D), jnp.uint32)
                    return pltpu.bitcast(wraw[i, pl.ds(r0, 16), :], jnp.uint32)
                lo, hi = [], []
                for jp in range(NTAP // 2):
                    ta, tb = tap(2 * jp), tap(2 * jp + 1)
                    lo.append(jnp.where(low, ta, pltpu.roll(tb, 4, 0)))
                    hi.append(jnp.where(low, pltpu.roll(ta, 4, 0), tb))
                lo = pltpu.bitcast(jnp.concatenate(lo, axis=0), jnp.bfloat16)
                hi = pltpu.bitcast(jnp.concatenate(hi, axis=0), jnp.bfloat16)
                rl = jnp.dot(g8, lo, preferred_element_type=jnp.float32)
                rh = jnp.dot(g8, hi, preferred_element_type=jnp.float32)
                for ri in range(2):
                    for k in range(NF):
                        r = (ri * NF + k) * 8
                        v = jnp.concatenate([rl[r:r + 8], rh[r:r + 8]], axis=0)
                        wt_ref[k, pl.ds(p * D + r0, 16), ri * D:(ri + 1) * D] = (
                            v.astype(jnp.bfloat16))
            return 0

        def piece(i, _):
            w_copy(i).wait()
            lax.fori_loop(i * (WPIECE // 16), (i + 1) * (WPIECE // 16), group, 0)
            return 0
        lax.fori_loop(0, NWP, piece, 0)

    def conv(b, dbuf, ybuf):
        href = hrefs[b]
        with jax.named_scope("xwait"):
            x_copy(b).wait()

        def fwd(q, _):
            f2 = f2_ref[...]
            r = pl.multiple_of(q * (4 * M_OUT), 16)
            x0 = xbuf[pl.ds(r, 2 * N), :]
            x1 = xbuf[pl.ds(r + 2 * M_OUT, 2 * N), :]
            r0 = jnp.dot(f2, x0, preferred_element_type=jnp.float32)
            r1 = jnp.dot(f2, x1, preferred_element_type=jnp.float32)
            pk = pltpu.pack_elementwise([r0, r1], packed_dtype=jnp.bfloat16)
            for p in range(2):
                for ri in range(2):
                    rr = (p * 2 + ri) * NF
                    for ct in range(CT):
                        dbuf[p * CT + ct, pl.ds(ri * NP + q, NF, stride=NB), :] = (
                            pk[rr:rr + NF, ct * 128:(ct + 1) * 128])
            return 0
        with jax.named_scope("fwd"):
            lax.fori_loop(0, NP, fwd, 0, unroll=6)

        if b + 1 < B:
            x_copy(b + 1).start()

        def mix(k, _):
            r = pl.multiple_of(k * NB, 8)
            lhs = jnp.concatenate(
                [dbuf[s, pl.ds(r, NB), :] for s in range(2 * CT)], axis=1)
            lhs = pltpu.bitcast(lhs, jnp.bfloat16)
            res = jnp.dot(lhs, wt_ref[k], preferred_element_type=jnp.float32)
            yr = res[:NB, :D] - res[NB:, D:]
            yi = res[:NB, D:] + res[NB:, :D]
            pk = pltpu.pack_elementwise([yr, yi], packed_dtype=jnp.bfloat16)
            for ct in range(CT):
                ybuf[ct, pl.ds(r, NB), :] = pk[:, ct * 128:(ct + 1) * 128]
            if b > 0:
                hp = hrefs[b - 1]
                GR = hp.shape[0] // NF
                mu_p = sc_ref[2 * b - 2:2 * b - 1, :]
                sc_p = sc_ref[2 * b - 1:2 * b, :]
                be = bet_ref[...].astype(jnp.float32)
                for c in range(GR // 64):
                    rows = pl.ds(pl.multiple_of(k * GR, 64) + c * 64, 64)
                    h = hp[rows, :].astype(jnp.float32)
                    hp[rows, :] = _gelu((h - mu_p) * sc_p + be).astype(hp.dtype)
            return 0
        with jax.named_scope("mix"):
            lax.fori_loop(0, NF, mix, 0)

        def inv(q):
            parts = []
            for s in range(2):
                parts.append(jnp.concatenate(
                    [ybuf[ct, pl.ds(2 * q + s, NF, stride=NB), :] for ct in range(CT)],
                    axis=1))
            rhs = pltpu.bitcast(jnp.concatenate(parts, axis=0), jnp.bfloat16)
            return jnp.dot(a2_ref[...], rhs, preferred_element_type=jnp.float32)

        def fold(y):
            acc = y[0:8]
            for i in range(1, y.shape[0] // 8):
                acc = acc + y[8 * i:8 * i + 8]
            return acc

        def stats(y, s1, s2, shift):
            d = y - shift
            return s1 + fold(d), s2 + fold(d * d)

        def inv_body(q, c):
            y = inv(q)
            href[pl.ds(pl.multiple_of(q * RP, 16), RP), :] = y.astype(href.dtype)
            return stats(y, c[0], c[1], shift)
        with jax.named_scope("inv"):
            y = inv(0)
            href[pl.ds(0, RP), :] = y.astype(href.dtype)
            shift = y[0:1]
            z = jnp.zeros((8, D), jnp.float32)
            c = stats(y, z, z, shift)
            s1, s2 = lax.fori_loop(1, nfull, inv_body, c, unroll=INV_UNROLL)
            for q in range(nfull, NP):
                y = inv(q)
                valid = lax.broadcasted_iota(jnp.int32, y.shape, 0) < (L - q * RP)
                href[pl.ds(q * RP, RP), :] = jnp.where(valid, y, 0.0).astype(href.dtype)
                s1, s2 = stats(jnp.where(valid, y, shift), s1, s2, shift)
        m1 = jnp.sum(s1, axis=0, keepdims=True) * np.float32(1.0 / L)
        m2 = jnp.sum(s2, axis=0, keepdims=True) * np.float32(1.0 / L)
        mu = shift + m1
        var = jnp.maximum(m2 - m1 * m1, 0.0)
        scale = lax.rsqrt(var + np.float32(1e-5)) * gam_ref[...].astype(jnp.float32)
        sc_ref[2 * b:2 * b + 1, :] = mu
        sc_ref[2 * b + 1:2 * b + 2, :] = scale

    @pl.when(j == 0)
    def _heavy():
        with jax.named_scope("weights"):
            pl.run_scoped(weights, pltpu.VMEM((K, D, D), jnp.bfloat16),
                          pltpu.SemaphoreType.DMA((NWP,)))
        for b in range(B):
            pl.run_scoped(functools.partial(conv, b),
                          pltpu.VMEM((2 * CT, NF * NB, 128), jnp.uint32),
                          pltpu.VMEM((CT, NF * NB, 128), jnp.uint32))

    beta = bet_ref[...].astype(jnp.float32)
    CH = 64

    def norm(i, _):
        r = pl.multiple_of(i * CH, CH)
        rows = pl.ds(pl.multiple_of(j * OUT_ROWS, OUT_ROWS) + r, CH)
        ys = []
        for b in range(B):
            h = hrefs[b][rows, :].astype(jnp.float32)
            if b + 1 == B:
                h = _gelu((h - sc_ref[2 * b:2 * b + 1, :]) * sc_ref[2 * b + 1:2 * b + 2, :] + beta)
            ys.append(h)
        pk = pltpu.pack_elementwise(ys, packed_dtype=jnp.bfloat16)
        o_ref[pl.ds(r, CH)] = pltpu.bitcast(pk.reshape(CH, 1, D), jnp.bfloat16)
        return 0
    with jax.named_scope("norm"):
        lax.fori_loop(0, OUT_ROWS // CH, norm, 0)


@jax.jit
def pallas_standalone__self_sup_conv_stem_wavlm__speech_kernel(
    x: jax.Array,
    w: jax.Array,
    gn_gamma: jax.Array,
    gn_beta: jax.Array,
):
    B, T, D = x.shape
    K = w.shape[0]
    L = (T - K) // 2 + 1
    assert B == 2 and (K + 1) // 2 <= NTAP and D % 128 == 0 and T % 16 == 0
    NB = -(-L // M_OUT)
    NB = -(-NB // 8) * 8
    NJ = -(-L // OUT_ROWS)
    hrows = -(-max(NB * M_OUT, NJ * OUT_ROWS) // (64 * NF)) * (64 * NF)
    xrows = 2 * M_OUT * (NB - 1) + 2 * N
    xrows = max(xrows, T + 16)
    f2, g8, a2 = _constants()
    dt = x.dtype
    consts = [jnp.asarray(c, dtype=jnp.bfloat16) for c in (f2, g8, a2)]

    def full(shape):
        return pl.BlockSpec(shape, lambda j: (0,) * len(shape))

    kern = functools.partial(_kernel, B=B, T=T, D=D, K=K, L=L, NB=NB)
    out = pl.pallas_call(
        kern,
        grid=(NJ,),
        in_specs=[
            pl.BlockSpec(memory_space=pl.ANY),
            pl.BlockSpec(memory_space=pl.ANY),
            full((1, D)), full((1, D)),
            full(f2.shape), full(g8.shape), full(a2.shape),
        ],
        out_specs=pl.BlockSpec((OUT_ROWS, B, D), lambda j: (j, 0, 0)),
        out_shape=jax.ShapeDtypeStruct((L, B, D), jnp.bfloat16),
        scratch_shapes=[
            pltpu.VMEM((NF, 2 * D, 2 * D), jnp.bfloat16),
            pltpu.VMEM((xrows, D), jnp.bfloat16),
            pltpu.VMEM((hrows, D), jnp.bfloat16),
            pltpu.VMEM((8, D), jnp.float32),
            pltpu.SemaphoreType.DMA((1,)),
        ],
        compiler_params=pltpu.CompilerParams(
            dimension_semantics=("arbitrary",),
            vmem_limit_bytes=126 * 1024 * 1024),
    )(x.astype(jnp.bfloat16), w.astype(jnp.bfloat16),
      gn_gamma.reshape(1, D), gn_beta.reshape(1, D), *consts)
    return jnp.transpose(out, (1, 0, 2)).astype(dt)
```

```python
import functools

import numpy as np
import jax
import jax.numpy as jnp
from jax import lax
import jax.experimental.pallas as pl
import jax.experimental.pallas.tpu as pltpu

N = 64
NF = N // 2
M_OUT = 48
NTAP = 16
INV_UNROLL = 4
MIX_UNROLL = 2
f32 = jnp.float32
OUT_ROWS = 256


def _constants():
    theta = 2.0 * np.pi * (np.arange(NF) + 0.5) / N
    t = np.arange(N)
    ang = theta[:, None] * t[None, :]
    fr = np.concatenate([np.cos(ang), -np.sin(ang)], axis=0)
    f2 = np.zeros((2, 2 * NF, N, 2), np.float32)
    for p in range(2):
        f2[p, :, :, p] = fr
    f2 = f2.reshape(4 * NF, 2 * N)
    j = np.arange(NTAP)
    ang = theta[:, None] * j[None, :]
    g = np.concatenate([np.cos(ang), np.sin(ang)], axis=0)
    g8 = np.kron(g, np.eye(8)).astype(np.float32)
    m = np.arange(M_OUT)
    ang = m[:, None] * theta[None, :]
    a = np.stack([np.cos(ang), -np.sin(ang)], axis=-1).reshape(M_OUT, N) * (2.0 / N)
    a2 = np.kron(np.eye(2), a).astype(np.float32)
    return f2, g8, a2


def _gelu(x):
    c = np.float32(np.sqrt(2.0 / np.pi))
    u = x * (c + (c * np.float32(0.044715)) * (x * x))
    hx = 0.5 * x
    return hx + hx * jnp.tanh(u)


def _kernel(x_hbm, w_hbm, gam_ref, bet_ref, f2_ref, g8_ref, a2_ref, o_hbm,
            wt_ref, xbuf, hbuf, sc_ref, xsem, *, B, T, D, K, L, NB):
    NP = NB // 2
    CT = D // 128
    WPIECE = 64
    NWP = D // WPIECE
    RP = 2 * M_OUT
    nfull = L // RP
    hrefs = (hbuf, xbuf)

    def x_copy(bb):
        return pltpu.make_async_copy(x_hbm.at[bb], xbuf.at[pl.ds(0, T)], xsem.at[0])

    def weights(wraw, wsem):
        def w_copy(i):
            return pltpu.make_async_copy(
                w_hbm.at[:, pl.ds(i * WPIECE, WPIECE), :],
                wraw.at[:, pl.ds(i * WPIECE, WPIECE), :], wsem.at[i])
        for i in range(NWP):
            w_copy(i).start()
        x_copy(0).start()
        xbuf[pl.ds(T, xbuf.shape[0] - T), :] = jnp.zeros(
            (xbuf.shape[0] - T, D), xbuf.dtype)
        if hbuf.shape[0] > NB * M_OUT:
            hbuf[pl.ds(NB * M_OUT, hbuf.shape[0] - NB * M_OUT), :] = jnp.zeros(
                (hbuf.shape[0] - NB * M_OUT, D), hbuf.dtype)

        low = lax.broadcasted_iota(jnp.int32, (8, D), 0) < 4

        def group(G, _):
            r0 = pl.multiple_of(G * 16, 16)
            g8 = g8_ref[...]
            for p in range(2):
                def tap(jj):
                    i = 2 * jj + p
                    if i >= K:
                        return jnp.zeros((8, D), jnp.uint32)
                    return pltpu.bitcast(wraw[i, pl.ds(r0, 16), :], jnp.uint32)
                lo, hi = [], []
                for jp in range(NTAP // 2):
                    ta, tb = tap(2 * jp), tap(2 * jp + 1)
                    lo.append(jnp.where(low, ta, pltpu.roll(tb, 4, 0)))
                    hi.append(jnp.where(low, pltpu.roll(ta, 4, 0), tb))
                lo = pltpu.bitcast(jnp.concatenate(lo, axis=0), jnp.bfloat16)
                hi = pltpu.bitcast(jnp.concatenate(hi, axis=0), jnp.bfloat16)
                rl = jnp.dot(g8, lo, preferred_element_type=jnp.float32)
                rh = jnp.dot(g8, hi, preferred_element_type=jnp.float32)
                for ri in range(2):
                    for k in range(NF):
                        r = (ri * NF + k) * 8
                        v = jnp.concatenate([rl[r:r + 8], rh[r:r + 8]], axis=0)
                        wt_ref[k, pl.ds(p * D + r0, 16), ri * D:(ri + 1) * D] = (
                            v.astype(jnp.bfloat16))
            return 0

        def piece(i, _):
            w_copy(i).wait()
            lax.fori_loop(i * (WPIECE // 16), (i + 1) * (WPIECE // 16), group, 0)
            return 0
        lax.fori_loop(0, NWP, piece, 0)

    def conv(b, dbuf, ybuf):
        href = hrefs[b]
        with jax.named_scope("xwait"):
            x_copy(b).wait()

        def fwd(q, _):
            f2 = f2_ref[...]
            r = pl.multiple_of(q * (4 * M_OUT), 16)
            x0 = xbuf[pl.ds(r, 2 * N), :]
            x1 = xbuf[pl.ds(r + 2 * M_OUT, 2 * N), :]
            r0 = jnp.dot(f2, x0, preferred_element_type=jnp.float32)
            r1 = jnp.dot(f2, x1, preferred_element_type=jnp.float32)
            pk = pltpu.pack_elementwise([r0, r1], packed_dtype=jnp.bfloat16)
            for p in range(2):
                for ri in range(2):
                    rr = (p * 2 + ri) * NF
                    for ct in range(CT):
                        dbuf[p * CT + ct, pl.ds(ri * NP + q, NF, stride=NB), :] = (
                            pk[rr:rr + NF, ct * 128:(ct + 1) * 128])
            return 0
        with jax.named_scope("fwd"):
            lax.fori_loop(0, NP, fwd, 0, unroll=6)

        if b + 1 < B:
            x_copy(b + 1).start()

        def mix(k, _):
            r = pl.multiple_of(k * NB, 8)
            lhs = jnp.concatenate(
                [dbuf[s, pl.ds(r, NB), :] for s in range(2 * CT)], axis=1)
            lhs = pltpu.bitcast(lhs, jnp.bfloat16)
            a, bb = lhs[:NB], lhs[NB:]
            c, d = wt_ref[k, :, :D], wt_ref[k, :, D:]
            ab = (a.astype(f32) + bb.astype(f32)).astype(jnp.bfloat16)
            cd = (c.astype(f32) + d.astype(f32)).astype(jnp.bfloat16)
            k1 = jnp.dot(a, c, preferred_element_type=f32)
            k2 = jnp.dot(bb, d, preferred_element_type=f32)
            k3 = jnp.dot(ab, cd, preferred_element_type=f32)
            yr = k1 - k2
            yi = k3 - k1 - k2
            pk = pltpu.pack_elementwise([yr, yi], packed_dtype=jnp.bfloat16)
            for ct in range(CT):
                ybuf[ct, pl.ds(r, NB), :] = pk[:, ct * 128:(ct + 1) * 128]
            if b > 0:
                hp = hrefs[b - 1]
                GR = hp.shape[0] // NF
                mu_p = sc_ref[2 * b - 2:2 * b - 1, :]
                sc_p = sc_ref[2 * b - 1:2 * b, :]
                be = bet_ref[...].astype(f32).reshape(1, D)
                for c in range(GR // 64):
                    rows = pl.ds(pl.multiple_of(k * GR, 64) + c * 64, 64)
                    h = hp[rows, :].astype(jnp.float32)
                    hp[rows, :] = _gelu((h - mu_p) * sc_p + be).astype(hp.dtype)
            return 0
        with jax.named_scope("mix"):
            lax.fori_loop(0, NF, mix, 0, unroll=MIX_UNROLL)

        def inv(q):
            parts = []
            for s in range(2):
                parts.append(jnp.concatenate(
                    [ybuf[ct, pl.ds(2 * q + s, NF, stride=NB), :] for ct in range(CT)],
                    axis=1))
            rhs = pltpu.bitcast(jnp.concatenate(parts, axis=0), jnp.bfloat16)
            return jnp.dot(a2_ref[...], rhs, preferred_element_type=jnp.float32)

        def fold(y):
            acc = y[0:8]
            for i in range(1, y.shape[0] // 8):
                acc = acc + y[8 * i:8 * i + 8]
            return acc

        def stats(y, s1, s2, shift):
            d = y - shift
            return s1 + fold(d), s2 + fold(d * d)

        def inv_body(q, c):
            y = inv(q)
            href[pl.ds(pl.multiple_of(q * RP, 16), RP), :] = y.astype(href.dtype)
            return stats(y, c[0], c[1], shift)
        with jax.named_scope("inv"):
            y = inv(0)
            href[pl.ds(0, RP), :] = y.astype(href.dtype)
            shift = y[0:1]
            z = jnp.zeros((8, D), jnp.float32)
            c = stats(y, z, z, shift)
            s1, s2 = lax.fori_loop(1, nfull, inv_body, c, unroll=INV_UNROLL)
            for q in range(nfull, NP):
                y = inv(q)
                valid = lax.broadcasted_iota(jnp.int32, y.shape, 0) < (L - q * RP)
                href[pl.ds(q * RP, RP), :] = jnp.where(valid, y, 0.0).astype(href.dtype)
                s1, s2 = stats(jnp.where(valid, y, shift), s1, s2, shift)
        m1 = jnp.sum(s1, axis=0, keepdims=True) * np.float32(1.0 / L)
        m2 = jnp.sum(s2, axis=0, keepdims=True) * np.float32(1.0 / L)
        mu = shift + m1
        var = jnp.maximum(m2 - m1 * m1, 0.0)
        scale = lax.rsqrt(var + np.float32(1e-5)) * gam_ref[...].astype(f32).reshape(1, D)
        sc_ref[2 * b:2 * b + 1, :] = mu
        sc_ref[2 * b + 1:2 * b + 2, :] = scale

    with jax.named_scope("weights"):
        pl.run_scoped(weights, pltpu.VMEM((K, D, D), jnp.bfloat16),
                      pltpu.SemaphoreType.DMA((NWP,)))
    for b in range(B):
        pl.run_scoped(functools.partial(conv, b),
                      pltpu.VMEM((2 * CT, NF * NB, 128), jnp.uint32),
                      pltpu.VMEM((CT, NF * NB, 128), jnp.uint32))

    def finish(ostage, osem):
        beta = bet_ref[...].astype(f32).reshape(1, D)
        CH = 64

        def rows_out(r, n):
            ys = []
            for b in range(B):
                h = hrefs[b][pl.ds(r, n), :].astype(f32)
                if b + 1 == B:
                    h = _gelu((h - sc_ref[2 * b:2 * b + 1, :]) * sc_ref[2 * b + 1:2 * b + 2, :]
                              + beta)
                ys.append(h)
            pk = pltpu.pack_elementwise(ys, packed_dtype=jnp.bfloat16)
            ostage[pl.ds(r, n)] = pltpu.bitcast(pk.reshape(n, 1, D), jnp.bfloat16)

        def o_copy(r, n):
            return pltpu.make_async_copy(ostage.at[pl.ds(r, n)], o_hbm.at[pl.ds(r, n)],
                                         osem.at[0])

        def chunk(i, _):
            r = pl.multiple_of(i * OUT_ROWS, OUT_ROWS)

            def sub(t, _):
                rows_out(pl.multiple_of(r + t * CH, CH), CH)
                return 0
            lax.fori_loop(0, OUT_ROWS // CH, sub, 0, unroll=2)
            o_copy(r, OUT_ROWS).start()
            return 0
        nch = L // OUT_ROWS
        lax.fori_loop(0, nch, chunk, 0, unroll=False)
        rem = L - nch * OUT_ROWS
        if rem:
            for t in range(-(-rem // CH)):
                rows_out(nch * OUT_ROWS + t * CH, CH)
            o_copy(nch * OUT_ROWS, rem).start()

        def wait(i, _):
            o_copy(pl.multiple_of(i * OUT_ROWS, OUT_ROWS), OUT_ROWS).wait()
            return 0
        lax.fori_loop(0, nch, wait, 0)
        if rem:
            o_copy(nch * OUT_ROWS, rem).wait()

    with jax.named_scope("finish"):
        pl.run_scoped(finish, pltpu.VMEM((hbuf.shape[0], B, D), jnp.bfloat16),
                      pltpu.SemaphoreType.DMA((1,)))


@jax.jit
def pallas_standalone__self_sup_conv_stem_wavlm__speech_kernel(
    x: jax.Array,
    w: jax.Array,
    gn_gamma: jax.Array,
    gn_beta: jax.Array,
):
    B, T, D = x.shape
    K = w.shape[0]
    L = (T - K) // 2 + 1
    assert B == 2 and (K + 1) // 2 <= NTAP and D % 128 == 0 and T % 16 == 0
    NB = -(-L // M_OUT)
    NB = -(-NB // 8) * 8
    NJ = -(-L // OUT_ROWS)
    hrows = -(-max(NB * M_OUT, NJ * OUT_ROWS) // (64 * NF)) * (64 * NF)
    xrows = 2 * M_OUT * (NB - 1) + 2 * N
    xrows = max(xrows, T + 16)
    f2, g8, a2 = _constants()
    dt = x.dtype
    consts = [jnp.asarray(c, dtype=jnp.bfloat16) for c in (f2, g8, a2)]

    vmem = pl.BlockSpec(memory_space=pltpu.VMEM)
    hbm = pl.BlockSpec(memory_space=pl.ANY)
    kern = functools.partial(_kernel, B=B, T=T, D=D, K=K, L=L, NB=NB)
    out = pl.pallas_call(
        kern,
        in_specs=[hbm, hbm, vmem, vmem, vmem, vmem, vmem],
        out_specs=hbm,
        out_shape=jax.ShapeDtypeStruct((L, B, D), jnp.bfloat16),
        scratch_shapes=[
            pltpu.VMEM((NF, 2 * D, 2 * D), jnp.bfloat16),
            pltpu.VMEM((xrows, D), jnp.bfloat16),
            pltpu.VMEM((hrows, D), jnp.bfloat16),
            pltpu.VMEM((8, D), f32),
            pltpu.SemaphoreType.DMA((1,)),
        ],
        compiler_params=pltpu.CompilerParams(vmem_limit_bytes=126 * 1024 * 1024),
    )(x.astype(jnp.bfloat16), w.astype(jnp.bfloat16), gn_gamma, gn_beta, *consts)
    return jnp.transpose(out, (1, 0, 2)).astype(dt)
```

```python
import functools

import numpy as np
import jax
import jax.numpy as jnp
from jax import lax
import jax.experimental.pallas as pl
import jax.experimental.pallas.tpu as pltpu

N = 64
NF = N // 2
M_OUT = 48
NTAP = 16
INV_UNROLL = 8
MIX_UNROLL = 4
FWD_UNROLL = 12
W_UNROLL = 2
WPIECE = 32
f32 = jnp.float32
OUT_ROWS = 256


def _constants():
    theta = 2.0 * np.pi * (np.arange(NF) + 0.5) / N
    t = np.arange(N)
    ang = theta[:, None] * t[None, :]
    fr = np.concatenate([np.cos(ang), -np.sin(ang)], axis=0)
    f2 = np.zeros((2, 2 * NF, N, 2), np.float32)
    for p in range(2):
        f2[p, :, :, p] = fr
    f2 = f2.reshape(4 * NF, 2 * N)
    j = np.arange(NTAP)
    ang = theta[:, None] * j[None, :]
    g = np.concatenate([np.cos(ang), np.sin(ang)], axis=0)
    g8 = np.kron(g, np.eye(8)).astype(np.float32)
    m = np.arange(M_OUT)
    ang = m[:, None] * theta[None, :]
    a = np.stack([np.cos(ang), -np.sin(ang)], axis=-1).reshape(M_OUT, N) * (2.0 / N)
    a2 = np.kron(np.eye(2), a).astype(np.float32)
    return f2, g8, a2


def _gelu(x):
    c = np.float32(np.sqrt(2.0 / np.pi))
    u = x * (c + (c * np.float32(0.044715)) * (x * x))
    hx = 0.5 * x
    return hx + hx * jnp.tanh(u)


def _kernel(x_hbm, w_hbm, gam_ref, bet_ref, f2_ref, g8_ref, a2_ref, o_hbm,
            wt_ref, xbuf, hbuf, sc_ref, xsem, *, B, T, D, K, L, NB):
    NP = NB // 2
    CT = D // 128
    NWP = D // WPIECE
    RP = 2 * M_OUT
    nfull = L // RP
    hrefs = (hbuf, xbuf)

    def x_copy(bb):
        return pltpu.make_async_copy(x_hbm.at[bb], xbuf.at[pl.ds(0, T)], xsem.at[0])

    def weights(wraw, wsem):
        def w_copy(i):
            return pltpu.make_async_copy(
                w_hbm.at[:, pl.ds(i * WPIECE, WPIECE), :],
                wraw.at[:, pl.ds(i * WPIECE, WPIECE), :], wsem.at[i])
        for i in range(NWP):
            w_copy(i).start()
        x_copy(0).start()
        xbuf[pl.ds(T, xbuf.shape[0] - T), :] = jnp.zeros(
            (xbuf.shape[0] - T, D), xbuf.dtype)
        if hbuf.shape[0] > NB * M_OUT:
            hbuf[pl.ds(NB * M_OUT, hbuf.shape[0] - NB * M_OUT), :] = jnp.zeros(
                (hbuf.shape[0] - NB * M_OUT, D), hbuf.dtype)

        low = lax.broadcasted_iota(jnp.int32, (8, D), 0) < 4

        def group(G, _):
            r0 = pl.multiple_of(G * 16, 16)
            g8 = g8_ref[...]
            for p in range(2):
                def tap(jj):
                    i = 2 * jj + p
                    if i >= K:
                        return jnp.zeros((8, D), jnp.uint32)
                    return pltpu.bitcast(wraw[i, pl.ds(r0, 16), :], jnp.uint32)
                lo, hi = [], []
                for jp in range(NTAP // 2):
                    ta, tb = tap(2 * jp), tap(2 * jp + 1)
                    lo.append(jnp.where(low, ta, pltpu.roll(tb, 4, 0)))
                    hi.append(jnp.where(low, pltpu.roll(ta, 4, 0), tb))
                lo = pltpu.bitcast(jnp.concatenate(lo, axis=0), jnp.bfloat16)
                hi = pltpu.bitcast(jnp.concatenate(hi, axis=0), jnp.bfloat16)
                rl = jnp.dot(g8, lo, preferred_element_type=jnp.float32)
                rh = jnp.dot(g8, hi, preferred_element_type=jnp.float32)
                for ri in range(2):
                    for k in range(NF):
                        r = (ri * NF + k) * 8
                        v = jnp.concatenate([rl[r:r + 8], rh[r:r + 8]], axis=0)
                        wt_ref[k, pl.ds(p * D + r0, 16), ri * D:(ri + 1) * D] = (
                            v.astype(jnp.bfloat16))
            return 0

        def piece(i, _):
            w_copy(i).wait()
            lax.fori_loop(0, WPIECE // 16,
                          lambda g, c: group(i * (WPIECE // 16) + g, c), 0, unroll=W_UNROLL)
            return 0
        lax.fori_loop(0, NWP, piece, 0)

    def conv(b, dbuf, ybuf):
        href = hrefs[b]
        with jax.named_scope("xwait"):
            x_copy(b).wait()

        def fwd(q, _):
            f2 = f2_ref[...]
            r = pl.multiple_of(q * (4 * M_OUT), 16)
            x0 = xbuf[pl.ds(r, 2 * N), :]
            x1 = xbuf[pl.ds(r + 2 * M_OUT, 2 * N), :]
            r0 = jnp.dot(f2, x0, preferred_element_type=jnp.float32)
            r1 = jnp.dot(f2, x1, preferred_element_type=jnp.float32)
            pk = pltpu.pack_elementwise([r0, r1], packed_dtype=jnp.bfloat16)
            for p in range(2):
                for ri in range(2):
                    rr = (p * 2 + ri) * NF
                    for ct in range(CT):
                        dbuf[p * CT + ct, pl.ds(ri * NP + q, NF, stride=NB), :] = (
                            pk[rr:rr + NF, ct * 128:(ct + 1) * 128])
            return 0
        with jax.named_scope("fwd"):
            lax.fori_loop(0, NP, fwd, 0, unroll=FWD_UNROLL)

        if b + 1 < B:
            x_copy(b + 1).start()

        def mix(k, _):
            r = pl.multiple_of(k * NB, 8)
            lhs = jnp.concatenate(
                [dbuf[s, pl.ds(r, NB), :] for s in range(2 * CT)], axis=1)
            lhs = pltpu.bitcast(lhs, jnp.bfloat16)
            a, bb = lhs[:NB], lhs[NB:]
            c, d = wt_ref[k, :, :D], wt_ref[k, :, D:]
            ab = (a.astype(f32) + bb.astype(f32)).astype(jnp.bfloat16)
            cd = (c.astype(f32) + d.astype(f32)).astype(jnp.bfloat16)
            k1 = jnp.dot(a, c, preferred_element_type=f32)
            k2 = jnp.dot(bb, d, preferred_element_type=f32)
            k3 = jnp.dot(ab, cd, preferred_element_type=f32)
            yr = k1 - k2
            yi = k3 - k1 - k2
            pk = pltpu.pack_elementwise([yr, yi], packed_dtype=jnp.bfloat16)
            for ct in range(CT):
                ybuf[ct, pl.ds(r, NB), :] = pk[:, ct * 128:(ct + 1) * 128]
            if b > 0:
                hp = hrefs[b - 1]
                GR = hp.shape[0] // NF
                mu_p = sc_ref[2 * b - 2:2 * b - 1, :]
                sc_p = sc_ref[2 * b - 1:2 * b, :]
                be = bet_ref[...].astype(f32).reshape(1, D)
                for c in range(GR // 64):
                    rows = pl.ds(pl.multiple_of(k * GR, 64) + c * 64, 64)
                    h = hp[rows, :].astype(jnp.float32)
                    hp[rows, :] = _gelu((h - mu_p) * sc_p + be).astype(hp.dtype)
            return 0
        with jax.named_scope("mix"):
            lax.fori_loop(0, NF, mix, 0, unroll=MIX_UNROLL)

        def inv(q):
            parts = []
            for s in range(2):
                parts.append(jnp.concatenate(
                    [ybuf[ct, pl.ds(2 * q + s, NF, stride=NB), :] for ct in range(CT)],
                    axis=1))
            rhs = pltpu.bitcast(jnp.concatenate(parts, axis=0), jnp.bfloat16)
            return jnp.dot(a2_ref[...], rhs, preferred_element_type=jnp.float32)

        def fold(y):
            acc = y[0:8]
            for i in range(1, y.shape[0] // 8):
                acc = acc + y[8 * i:8 * i + 8]
            return acc

        def stats(y, s1, s2, shift):
            d = y - shift
            return s1 + fold(d), s2 + fold(d * d)

        def inv_body(q, c):
            y = inv(q)
            href[pl.ds(pl.multiple_of(q * RP, 16), RP), :] = y.astype(href.dtype)
            return stats(y, c[0], c[1], shift)
        with jax.named_scope("inv"):
            y = inv(0)
            href[pl.ds(0, RP), :] = y.astype(href.dtype)
            shift = y[0:1]
            z = jnp.zeros((8, D), jnp.float32)
            c = stats(y, z, z, shift)
            s1, s2 = lax.fori_loop(1, nfull, inv_body, c, unroll=INV_UNROLL)
            for q in range(nfull, NP):
                y = inv(q)
                valid = lax.broadcasted_iota(jnp.int32, y.shape, 0) < (L - q * RP)
                href[pl.ds(q * RP, RP), :] = jnp.where(valid, y, 0.0).astype(href.dtype)
                s1, s2 = stats(jnp.where(valid, y, shift), s1, s2, shift)
        m1 = jnp.sum(s1, axis=0, keepdims=True) * np.float32(1.0 / L)
        m2 = jnp.sum(s2, axis=0, keepdims=True) * np.float32(1.0 / L)
        mu = shift + m1
        var = jnp.maximum(m2 - m1 * m1, 0.0)
        scale = lax.rsqrt(var + np.float32(1e-5)) * gam_ref[...].astype(f32).reshape(1, D)
        sc_ref[2 * b:2 * b + 1, :] = mu
        sc_ref[2 * b + 1:2 * b + 2, :] = scale

    with jax.named_scope("weights"):
        pl.run_scoped(weights, pltpu.VMEM((K, D, D), jnp.bfloat16),
                      pltpu.SemaphoreType.DMA((NWP,)))
    for b in range(B):
        pl.run_scoped(functools.partial(conv, b),
                      pltpu.VMEM((2 * CT, NF * NB, 128), jnp.uint32),
                      pltpu.VMEM((CT, NF * NB, 128), jnp.uint32))

    def finish(ostage, osem):
        beta = bet_ref[...].astype(f32).reshape(1, D)
        CH = 64

        def rows_out(r, n):
            ys = []
            for b in range(B):
                h = hrefs[b][pl.ds(r, n), :].astype(f32)
                if b + 1 == B:
                    h = _gelu((h - sc_ref[2 * b:2 * b + 1, :]) * sc_ref[2 * b + 1:2 * b + 2, :]
                              + beta)
                ys.append(h)
            pk = pltpu.pack_elementwise(ys, packed_dtype=jnp.bfloat16)
            ostage.bitcast(jnp.uint32)[pl.ds(r, n), 0, :] = pk

        def o_copy(r, n):
            return pltpu.make_async_copy(ostage.at[pl.ds(r, n)], o_hbm.at[pl.ds(r, n)],
                                         osem.at[0])

        def chunk(i, _):
            r = pl.multiple_of(i * OUT_ROWS, OUT_ROWS)

            def sub(t, _):
                rows_out(pl.multiple_of(r + t * CH, CH), CH)
                return 0
            lax.fori_loop(0, OUT_ROWS // CH, sub, 0, unroll=2)
            o_copy(r, OUT_ROWS).start()
            return 0
        nch = L // OUT_ROWS
        lax.fori_loop(0, nch, chunk, 0, unroll=False)
        rem = L - nch * OUT_ROWS
        if rem:
            for t in range(-(-rem // CH)):
                rows_out(nch * OUT_ROWS + t * CH, CH)
            o_copy(nch * OUT_ROWS, rem).start()

        def wait(i, _):
            o_copy(pl.multiple_of(i * OUT_ROWS, OUT_ROWS), OUT_ROWS).wait()
            return 0
        lax.fori_loop(0, nch, wait, 0)
        if rem:
            o_copy(nch * OUT_ROWS, rem).wait()

    with jax.named_scope("finish"):
        pl.run_scoped(finish, pltpu.VMEM((hbuf.shape[0], B, D), jnp.bfloat16),
                      pltpu.SemaphoreType.DMA((1,)))


@jax.jit
def pallas_standalone__self_sup_conv_stem_wavlm__speech_kernel(
    x: jax.Array,
    w: jax.Array,
    gn_gamma: jax.Array,
    gn_beta: jax.Array,
):
    B, T, D = x.shape
    K = w.shape[0]
    L = (T - K) // 2 + 1
    assert B == 2 and (K + 1) // 2 <= NTAP and D % 128 == 0 and T % 16 == 0
    NB = -(-L // M_OUT)
    NB = -(-NB // 8) * 8
    NJ = -(-L // OUT_ROWS)
    hrows = -(-max(NB * M_OUT, NJ * OUT_ROWS) // (64 * NF)) * (64 * NF)
    xrows = 2 * M_OUT * (NB - 1) + 2 * N
    xrows = max(xrows, T + 16)
    f2, g8, a2 = _constants()
    dt = x.dtype
    consts = [jnp.asarray(c, dtype=jnp.bfloat16) for c in (f2, g8, a2)]

    vmem = pl.BlockSpec(memory_space=pltpu.VMEM)
    hbm = pl.BlockSpec(memory_space=pl.ANY)
    kern = functools.partial(_kernel, B=B, T=T, D=D, K=K, L=L, NB=NB)
    out = pl.pallas_call(
        kern,
        in_specs=[hbm, hbm, vmem, vmem, vmem, vmem, vmem],
        out_specs=hbm,
        out_shape=jax.ShapeDtypeStruct((L, B, D), jnp.bfloat16),
        scratch_shapes=[
            pltpu.VMEM((NF, 2 * D, 2 * D), jnp.bfloat16),
            pltpu.VMEM((xrows, D), jnp.bfloat16),
            pltpu.VMEM((hrows, D), jnp.bfloat16),
            pltpu.VMEM((8, D), f32),
            pltpu.SemaphoreType.DMA((1,)),
        ],
        compiler_params=pltpu.CompilerParams(vmem_limit_bytes=126 * 1024 * 1024),
    )(x.astype(jnp.bfloat16), w.astype(jnp.bfloat16), gn_gamma, gn_beta, *consts)
    return jnp.transpose(out, (1, 0, 2)).astype(dt)
```

```python
import functools

import numpy as np
import jax
import jax.numpy as jnp
from jax import lax
import jax.experimental.pallas as pl
import jax.experimental.pallas.tpu as pltpu

N = 63
NF = 32
KP = 64
M_OUT = 48
NTAP = 16
SLAB_PAD = 8
NSEG = 7
INV_UNROLL = 8
MIX_UNROLL = 2
W_UNROLL = 2
WPIECE = 32
OUT_ROWS = 256
f32 = jnp.float32
bf16 = jnp.bfloat16


def _constants():
    theta = 2.0 * np.pi * (np.arange(NF) + 0.5) / N
    def cs(n):
        ang = theta[:, None] * np.arange(n)[None, :]
        c, s = np.cos(ang), np.sin(ang)
        s[NF - 1] = 0.0
        return c, s
    c, s = cs(N)
    fr = np.zeros((2 * NF, KP), np.float32)
    fr[:, :N] = np.concatenate([c, -s], axis=0)
    f2 = np.zeros((2, 2 * NF, KP, 2), np.float32)
    for p in range(2):
        f2[p, :, :, p] = fr
    f2 = f2.reshape(4 * NF, 2 * KP)
    c, s = cs(NTAP)
    g8 = np.kron(np.concatenate([c, s], axis=0), np.eye(8)).astype(np.float32)
    c, s = cs(M_OUT)
    wgt = np.full((NF, 1), 2.0 / N)
    wgt[NF - 1] = 1.0 / N
    a = np.stack([(c * wgt).T, (-s * wgt).T], axis=-1).reshape(M_OUT, 2 * NF)
    a2 = np.kron(np.eye(2), a).astype(np.float32)
    return f2, g8, a2


def _gelu(x):
    c = np.float32(np.sqrt(2.0 / np.pi))
    u = x * (c + (c * np.float32(0.044715)) * (x * x))
    hx = 0.5 * x
    return hx + hx * jnp.tanh(u)


def _kernel(x_hbm, w_hbm, gam_ref, bet_ref, f2_ref, g8_ref, a2_ref, o_hbm,
            xbuf, sc_ref, xsem, *, B, T, D, K, L, NB, HROWS):
    NP = NB // 2
    SEG = NP // NSEG
    XR = 4 * M_OUT * SEG
    MB = B * NB
    MS = MB + SLAB_PAD
    CT = D // 128
    NWP = D // WPIECE
    RP = 2 * M_OUT
    nfull = L // RP

    def x_copy(b, i, last=False):
        r = i * XR if last else pl.multiple_of(i * XR, 16)
        n = T - (NSEG - 1) * XR if last else XR
        return pltpu.make_async_copy(x_hbm.at[b, pl.ds(r, n)], xbuf.at[pl.ds(r, n)], xsem.at[i])

    def weights(wt_ref, wraw, wsem):
        def w_copy(i):
            return pltpu.make_async_copy(
                w_hbm.at[:, pl.ds(i * WPIECE, WPIECE), :],
                wraw.at[:, pl.ds(i * WPIECE, WPIECE), :], wsem.at[i])
        for i in range(NWP):
            w_copy(i).start()
        for i in range(NSEG):
            x_copy(0, i, i == NSEG - 1).start()
        xbuf[pl.ds(T, xbuf.shape[0] - T), :] = jnp.zeros((xbuf.shape[0] - T, D), bf16)

        low = lax.broadcasted_iota(jnp.int32, (8, D), 0) < 4

        def group(G):
            r0 = pl.multiple_of(G * 16, 16)
            g8 = g8_ref[...]
            for p in range(2):
                def tap(jj):
                    i = 2 * jj + p
                    if i >= K:
                        return jnp.zeros((8, D), jnp.uint32)
                    return pltpu.bitcast(wraw[i, pl.ds(r0, 16), :], jnp.uint32)
                lo, hi = [], []
                for jp in range(NTAP // 2):
                    ta, tb = tap(2 * jp), tap(2 * jp + 1)
                    lo.append(jnp.where(low, ta, pltpu.roll(tb, 4, 0)))
                    hi.append(jnp.where(low, pltpu.roll(ta, 4, 0), tb))
                lo = pltpu.bitcast(jnp.concatenate(lo, axis=0), bf16)
                hi = pltpu.bitcast(jnp.concatenate(hi, axis=0), bf16)
                rl = jnp.dot(g8, lo, preferred_element_type=f32)
                rh = jnp.dot(g8, hi, preferred_element_type=f32)
                for ri in range(2):
                    for k in range(NF - ri):
                        r = (ri * NF + k) * 8
                        v = jnp.concatenate([rl[r:r + 8], rh[r:r + 8]], axis=0)
                        wt_ref[k, pl.ds(p * D + r0, 16), ri * D:(ri + 1) * D] = v.astype(bf16)

        def piece(i, _):
            w_copy(i).wait()

            def inner(g, _):
                group(i * (WPIECE // 16) + g)
                return 0
            lax.fori_loop(0, WPIECE // 16, inner, 0, unroll=W_UNROLL)
            return 0
        lax.fori_loop(0, NWP, piece, 0)

    def fwd_mix(wt_ref, dlo, dhi):
        def fwd(b, q):
            f2 = f2_ref[...]
            r = pl.multiple_of(q * (4 * M_OUT), 16)
            r0 = jnp.dot(f2, xbuf[pl.ds(r, 2 * KP), :], preferred_element_type=f32)
            r1 = jnp.dot(f2, xbuf[pl.ds(r + 2 * M_OUT, 2 * KP), :], preferred_element_type=f32)
            pk = pltpu.pack_elementwise([r0, r1], packed_dtype=bf16)
            for p, dst in enumerate((dlo, dhi)):
                for ri in range(2):
                    rr = (p * 2 + ri) * NF
                    for ct in range(CT):
                        dst[ct, pl.ds(ri * (MB // 2) + b * NP + q, NF, stride=MS), :] = (
                            pk[rr:rr + NF, ct * 128:(ct + 1) * 128])

        def fwd_seg(b, i):
            def body(q, _):
                fwd(b, i * SEG + q)
                return 0
            lax.fori_loop(0, SEG, body, 0, unroll=True)

        def fwd_batch(b, _):
            x_copy(b, 0).wait()

            def seg(i, _):
                @pl.when(i + 1 < NSEG - 1)
                def _():
                    x_copy(b, i + 1).wait()

                @pl.when(i + 1 == NSEG - 1)
                def _():
                    x_copy(b, NSEG - 1, True).wait()
                fwd_seg(b, i)

                @pl.when((b + 1 < B) & (i < NSEG - 1))
                def _():
                    x_copy(b + 1, i).start()

                @pl.when((b + 1 < B) & (i == NSEG - 1))
                def _():
                    x_copy(b + 1, NSEG - 1, True).start()
                return 0
            lax.fori_loop(0, NSEG, seg, 0)
            return 0
        with jax.named_scope("fwd"):
            lax.fori_loop(0, B, fwd_batch, 0)

        def load_lhs(r):
            lhs = jnp.concatenate(
                [d[ct, pl.ds(r, MB), :] for d in (dlo, dhi) for ct in range(CT)], axis=1)
            return pltpu.bitcast(lhs, bf16)

        def store_y(r, yr, yi):
            pk = pltpu.pack_elementwise([yr, yi], packed_dtype=bf16)
            for ct in range(CT):
                dlo[ct, pl.ds(r, MB), :] = pk[:, ct * 128:(ct + 1) * 128]

        def mix(k, _):
            r = pl.multiple_of(k * MS, 8)
            lhs = load_lhs(r)
            a, bb = lhs[:MB], lhs[MB:]
            c, d = wt_ref[k, :, :D], wt_ref[k, :, D:]
            ab = (a.astype(f32) + bb.astype(f32)).astype(bf16)
            cd = (c.astype(f32) + d.astype(f32)).astype(bf16)
            k1 = jnp.dot(a, c, preferred_element_type=f32)
            k2 = jnp.dot(bb, d, preferred_element_type=f32)
            k3 = jnp.dot(ab, cd, preferred_element_type=f32)
            store_y(r, k1 - k2, k3 - k1 - k2)
            return 0
        with jax.named_scope("mix"):
            lax.fori_loop(0, NF - 1, mix, 0, unroll=MIX_UNROLL)
            r = (NF - 1) * MS
            k1 = jnp.dot(load_lhs(r)[:MB], wt_ref[NF - 1, :, :D], preferred_element_type=f32)
            store_y(r, k1, jnp.zeros_like(k1))

    def fold(y):
        acc = y[0:8]
        for i in range(1, y.shape[0] // 8):
            acc = acc + y[8 * i:8 * i + 8]
        return acc

    def inverse(ybuf, hbuf, b):
        def inv(q):
            parts = [jnp.concatenate(
                [ybuf[ct, pl.ds(b * NB + 2 * q + s, NF, stride=MS), :] for ct in range(CT)],
                axis=1) for s in range(2)]
            rhs = pltpu.bitcast(jnp.concatenate(parts, axis=0), bf16)
            return jnp.dot(a2_ref[...], rhs, preferred_element_type=f32)

        def stats(y, s1, s2, shift):
            d = y - shift
            return s1 + fold(d), s2 + fold(d * d)

        y = inv(0)
        hbuf[b, pl.ds(0, RP), :] = y.astype(bf16)
        shift = y[0:1]
        z = jnp.zeros((8, D), f32)
        c = stats(y, z, z, shift)

        def inv_body(q, c):
            y = inv(q)
            hbuf[b, pl.ds(pl.multiple_of(q * RP, 16), RP), :] = y.astype(bf16)
            return stats(y, c[0], c[1], shift)
        s1, s2 = lax.fori_loop(1, nfull, inv_body, c, unroll=INV_UNROLL)
        for q in range(nfull, NP):
            y = inv(q)
            valid = lax.broadcasted_iota(jnp.int32, y.shape, 0) < (L - q * RP)
            hbuf[b, pl.ds(q * RP, RP), :] = jnp.where(valid, y, 0.0).astype(bf16)
            s1, s2 = stats(jnp.where(valid, y, shift), s1, s2, shift)
        m1 = jnp.sum(s1, axis=0, keepdims=True) * np.float32(1.0 / L)
        m2 = jnp.sum(s2, axis=0, keepdims=True) * np.float32(1.0 / L)
        var = jnp.maximum(m2 - m1 * m1, 0.0)
        sc_ref[2 * b:2 * b + 1, :] = shift + m1
        sc_ref[2 * b + 1:2 * b + 2, :] = (
            lax.rsqrt(var + np.float32(1e-5)) * gam_ref[...].astype(f32).reshape(1, D))

    def tail(ybuf, hbuf, ostage, osem):
        with jax.named_scope("inv"):
            for b in range(B):
                inverse(ybuf, hbuf, b)
        beta = bet_ref[...].astype(f32).reshape(1, D)
        CH = 32
        o32 = ostage.bitcast(jnp.uint32)

        def rows_out(r):
            ys = []
            for b in range(B):
                h = hbuf[b, pl.ds(r, CH), :].astype(f32)
                ys.append(_gelu((h - sc_ref[2 * b:2 * b + 1, :]) * sc_ref[2 * b + 1:2 * b + 2, :]
                                + beta))
            o32[pl.ds(r, CH), 0, :] = pltpu.pack_elementwise(ys, packed_dtype=bf16)

        def o_copy(r, n):
            return pltpu.make_async_copy(ostage.at[pl.ds(r, n)], o_hbm.at[pl.ds(r, n)],
                                         osem.at[0])

        def chunk(i, _):
            r = pl.multiple_of(i * OUT_ROWS, OUT_ROWS)

            def sub(t, _):
                rows_out(pl.multiple_of(r + t * CH, CH))
                return 0
            lax.fori_loop(0, OUT_ROWS // CH, sub, 0, unroll=2)
            o_copy(r, OUT_ROWS).start()
            return 0

        def wait(i, _):
            o_copy(pl.multiple_of(i * OUT_ROWS, OUT_ROWS), OUT_ROWS).wait()
            return 0

        nch = L // OUT_ROWS
        rem = L - nch * OUT_ROWS
        with jax.named_scope("finish"):
            lax.fori_loop(0, nch, chunk, 0)
            if rem:
                for t in range(-(-rem // CH)):
                    rows_out(nch * OUT_ROWS + t * CH)
                o_copy(nch * OUT_ROWS, rem).start()
            lax.fori_loop(0, nch, wait, 0)
            if rem:
                o_copy(nch * OUT_ROWS, rem).wait()

    dshape = pltpu.VMEM((CT, NF * MS, 128), jnp.uint32)

    def main(dlo):
        def front(wt_ref):
            with jax.named_scope("weights"):
                pl.run_scoped(functools.partial(weights, wt_ref),
                              pltpu.VMEM((K, D, D), bf16), pltpu.SemaphoreType.DMA((NWP,)))
            pl.run_scoped(functools.partial(fwd_mix, wt_ref, dlo), dshape)
        pl.run_scoped(front, pltpu.VMEM((NF, 2 * D, 2 * D), bf16))
        pl.run_scoped(functools.partial(tail, dlo),
                      pltpu.VMEM((B, HROWS, D), bf16), pltpu.VMEM((HROWS, B, D), bf16),
                      pltpu.SemaphoreType.DMA((1,)))
    pl.run_scoped(main, dshape)


@jax.jit
def pallas_standalone__self_sup_conv_stem_wavlm__speech_kernel(
    x: jax.Array,
    w: jax.Array,
    gn_gamma: jax.Array,
    gn_beta: jax.Array,
):
    B, T, D = x.shape
    K = w.shape[0]
    L = (T - K) // 2 + 1
    assert B == 2 and (K + 1) // 2 <= NTAP and D % 128 == 0 and T % 16 == 0
    NB = -(-L // M_OUT)
    NB = -(-NB // (2 * NSEG)) * (2 * NSEG)
    assert (B * NB) % 16 == 0
    hrows = NB * M_OUT
    xrows = max(2 * M_OUT * (NB - 1) + 2 * KP, T + 16)
    assert (NSEG - 1) * (NB // NSEG) * 2 * M_OUT < T <= NB * 2 * M_OUT
    f2, g8, a2 = _constants()
    dt = x.dtype
    consts = [jnp.asarray(c, dtype=jnp.bfloat16) for c in (f2, g8, a2)]

    vmem = pl.BlockSpec(memory_space=pltpu.VMEM)
    hbm = pl.BlockSpec(memory_space=pl.ANY)
    kern = functools.partial(_kernel, B=B, T=T, D=D, K=K, L=L, NB=NB, HROWS=hrows)
    out = pl.pallas_call(
        kern,
        in_specs=[hbm, hbm, vmem, vmem, vmem, vmem, vmem],
        out_specs=hbm,
        out_shape=jax.ShapeDtypeStruct((L, B, D), jnp.bfloat16),
        scratch_shapes=[
            pltpu.VMEM((xrows, D), bf16),
            pltpu.VMEM((8, D), f32),
            pltpu.SemaphoreType.DMA((NSEG,)),
        ],
        compiler_params=pltpu.CompilerParams(vmem_limit_bytes=127 * 1024 * 1024 + 512 * 1024),
    )(x.astype(jnp.bfloat16), w.astype(jnp.bfloat16), gn_gamma, gn_beta, *consts)
    return jnp.transpose(out, (1, 0, 2)).astype(dt)
```

```python
import functools

import numpy as np
import jax
import jax.numpy as jnp
from jax import lax
import jax.experimental.pallas as pl
import jax.experimental.pallas.tpu as pltpu

N = 63
NF = 32
KP = 64
M_OUT = 48
NTAP = 16
SLAB_PAD = 4
NSEG = 6
INV_UNROLL = 27
MIX_UNROLL = 5
W_UNROLL = 2
WPIECE = 32
OUT_ROWS = 128
f32 = jnp.float32
bf16 = jnp.bfloat16


def _constants():
    theta = 2.0 * np.pi * (np.arange(NF) + 0.5) / N
    def cs(n):
        ang = theta[:, None] * np.arange(n)[None, :]
        c, s = np.cos(ang), np.sin(ang)
        s[NF - 1] = 0.0
        return c, s
    c, s = cs(N)
    fr = np.zeros((2 * NF, KP), np.float32)
    fr[:, :N] = np.concatenate([c, -s], axis=0)
    f2 = np.zeros((2, 2 * NF, KP, 2), np.float32)
    for p in range(2):
        f2[p, :, :, p] = fr
    f2 = f2.reshape(4 * NF, 2 * KP)
    c, s = cs(NTAP)
    g8 = np.kron(np.concatenate([c, s], axis=0), np.eye(8)).astype(np.float32)
    c, s = cs(M_OUT)
    wgt = np.full((NF, 1), 2.0 / N)
    wgt[NF - 1] = 1.0 / N
    a = np.stack([(c * wgt).T, (-s * wgt).T], axis=-1).reshape(M_OUT, 2 * NF)
    a2 = np.kron(np.eye(2), a).astype(np.float32)
    return f2, g8, a2


def _gelu(x):
    c = np.float32(np.sqrt(2.0 / np.pi))
    u = x * (c + (c * np.float32(0.044715)) * (x * x))
    hx = 0.5 * x
    return hx + hx * jnp.tanh(u)


def _kernel(x_hbm, w_hbm, gam_ref, bet_ref, f2_ref, g8_ref, a2_ref, o_hbm,
            xbuf, sc_ref, xsem, *, B, T, D, K, L, NB, HROWS):
    NP = NB // 2
    SEG = NP // NSEG
    XR = 4 * M_OUT * SEG
    MB = B * NB
    MS = MB + SLAB_PAD
    CT = D // 128
    NWP = D // WPIECE
    RP = 2 * M_OUT
    nfull = L // RP

    def x_copy(b, i, last=False):
        r = i * XR if last else pl.multiple_of(i * XR, 16)
        n = T - (NSEG - 1) * XR if last else XR
        return pltpu.make_async_copy(x_hbm.at[b, pl.ds(r, n)], xbuf.at[pl.ds(r, n)], xsem.at[i])

    def weights(wt_ref, wraw, wsem):
        def w_copy(i):
            return pltpu.make_async_copy(
                w_hbm.at[:, pl.ds(i * WPIECE, WPIECE), :],
                wraw.at[:, pl.ds(i * WPIECE, WPIECE), :], wsem.at[i])
        for i in range(NWP):
            w_copy(i).start()
        for i in range(NSEG):
            x_copy(0, i, i == NSEG - 1).start()
        xbuf[pl.ds(T, xbuf.shape[0] - T), :] = jnp.zeros((xbuf.shape[0] - T, D), bf16)

        low = lax.broadcasted_iota(jnp.int32, (8, D), 0) < 4

        def group(G):
            r0 = pl.multiple_of(G * 16, 16)
            g8 = g8_ref[...]
            for p in range(2):
                def tap(jj):
                    i = 2 * jj + p
                    if i >= K:
                        return jnp.zeros((8, D), jnp.uint32)
                    return pltpu.bitcast(wraw[i, pl.ds(r0, 16), :], jnp.uint32)
                lo, hi = [], []
                for jp in range(NTAP // 2):
                    ta, tb = tap(2 * jp), tap(2 * jp + 1)
                    lo.append(jnp.where(low, ta, pltpu.roll(tb, 4, 0)))
                    hi.append(jnp.where(low, pltpu.roll(ta, 4, 0), tb))
                lo = pltpu.bitcast(jnp.concatenate(lo, axis=0), bf16)
                hi = pltpu.bitcast(jnp.concatenate(hi, axis=0), bf16)
                rl = jnp.dot(g8, lo, preferred_element_type=f32)
                rh = jnp.dot(g8, hi, preferred_element_type=f32)
                for ri in range(2):
                    for k in range(NF - ri):
                        r = (ri * NF + k) * 8
                        v = jnp.concatenate([rl[r:r + 8], rh[r:r + 8]], axis=0)
                        wt_ref[k, pl.ds(p * D + r0, 16), ri * D:(ri + 1) * D] = v.astype(bf16)

        def piece(i, _):
            w_copy(i).wait()

            def inner(g, _):
                group(i * (WPIECE // 16) + g)
                return 0
            lax.fori_loop(0, WPIECE // 16, inner, 0, unroll=W_UNROLL)
            return 0
        lax.fori_loop(0, NWP, piece, 0)

    def fwd_mix(wt_ref, dlo, dhi):
        def fwd(b, q):
            f2 = f2_ref[...]
            r = pl.multiple_of(q * (4 * M_OUT), 16)
            r0 = jnp.dot(f2, xbuf[pl.ds(r, 2 * KP), :], preferred_element_type=f32)
            r1 = jnp.dot(f2, xbuf[pl.ds(r + 2 * M_OUT, 2 * KP), :], preferred_element_type=f32)
            pk = pltpu.pack_elementwise([r0, r1], packed_dtype=bf16)
            for p, dst in enumerate((dlo, dhi)):
                for ri in range(2):
                    rr = (p * 2 + ri) * NF
                    for ct in range(CT):
                        dst[ct, pl.ds(ri * (MB // 2) + b * NP + q, NF, stride=MS), :] = (
                            pk[rr:rr + NF, ct * 128:(ct + 1) * 128])

        def fwd_seg(b, i):
            def body(q, _):
                fwd(b, i * SEG + q)
                return 0
            lax.fori_loop(0, SEG, body, 0, unroll=True)

        def fwd_batch(b, _):
            x_copy(b, 0).wait()

            def seg(i, _):
                @pl.when(i + 1 < NSEG - 1)
                def _():
                    x_copy(b, i + 1).wait()

                @pl.when(i + 1 == NSEG - 1)
                def _():
                    x_copy(b, NSEG - 1, True).wait()
                fwd_seg(b, i)

                @pl.when((b + 1 < B) & (i < NSEG - 1))
                def _():
                    x_copy(b + 1, i).start()

                @pl.when((b + 1 < B) & (i == NSEG - 1))
                def _():
                    x_copy(b + 1, NSEG - 1, True).start()
                return 0
            lax.fori_loop(0, NSEG, seg, 0)
            return 0
        with jax.named_scope("fwd"):
            lax.fori_loop(0, B, fwd_batch, 0)

        def load_lhs(r):
            lhs = jnp.concatenate(
                [d[ct, pl.ds(r, MB), :] for d in (dlo, dhi) for ct in range(CT)], axis=1)
            return pltpu.bitcast(lhs, bf16)

        def store_y(r, yr, yi):
            pk = pltpu.pack_elementwise([yr, yi], packed_dtype=bf16)
            for ct in range(CT):
                dlo[ct, pl.ds(r, MB), :] = pk[:, ct * 128:(ct + 1) * 128]

        def mix(k, _):
            r = k * MS
            lhs = load_lhs(r)
            a, bb = lhs[:MB], lhs[MB:]
            c, d = wt_ref[k, :, :D], wt_ref[k, :, D:]
            ab = (a.astype(f32) + bb.astype(f32)).astype(bf16)
            cd = (c.astype(f32) + d.astype(f32)).astype(bf16)
            k1 = jnp.dot(a, c, preferred_element_type=f32)
            k2 = jnp.dot(bb, d, preferred_element_type=f32)
            k3 = jnp.dot(ab, cd, preferred_element_type=f32)
            store_y(r, k1 - k2, k3 - k1 - k2)
            return 0
        with jax.named_scope("mix"):
            lax.fori_loop(0, NF - 1, mix, 0, unroll=MIX_UNROLL)
            r = (NF - 1) * MS
            k1 = jnp.dot(load_lhs(r)[:MB], wt_ref[NF - 1, :, :D], preferred_element_type=f32)
            store_y(r, k1, jnp.zeros_like(k1))

    def fold(y):
        acc = y[0:8]
        for i in range(1, y.shape[0] // 8):
            acc = acc + y[8 * i:8 * i + 8]
        return acc

    def inverse(ybuf, hbuf, b):
        def inv(q):
            parts = [jnp.concatenate(
                [ybuf[ct, pl.ds(b * NB + 2 * q + s, NF, stride=MS), :] for ct in range(CT)],
                axis=1) for s in range(2)]
            rhs = pltpu.bitcast(jnp.concatenate(parts, axis=0), bf16)
            return jnp.dot(a2_ref[...], rhs, preferred_element_type=f32)

        def stats(y, s1, s2, shift):
            d = y - shift
            return s1 + fold(d), s2 + fold(d * d)

        y = inv(0)
        hbuf[b, pl.ds(0, RP), :] = y.astype(bf16)
        shift = y[0:1]
        z = jnp.zeros((8, D), f32)
        c = stats(y, z, z, shift)

        def inv_body(q, c):
            y = inv(q)
            hbuf[b, pl.ds(pl.multiple_of(q * RP, 16), RP), :] = y.astype(bf16)
            return stats(y, c[0], c[1], shift)
        s1, s2 = lax.fori_loop(1, nfull, inv_body, c, unroll=INV_UNROLL)
        for q in range(nfull, NP):
            y = inv(q)
            valid = lax.broadcasted_iota(jnp.int32, y.shape, 0) < (L - q * RP)
            hbuf[b, pl.ds(q * RP, RP), :] = jnp.where(valid, y, 0.0).astype(bf16)
            s1, s2 = stats(jnp.where(valid, y, shift), s1, s2, shift)
        m1 = jnp.sum(s1, axis=0, keepdims=True) * np.float32(1.0 / L)
        m2 = jnp.sum(s2, axis=0, keepdims=True) * np.float32(1.0 / L)
        var = jnp.maximum(m2 - m1 * m1, 0.0)
        sc_ref[2 * b:2 * b + 1, :] = shift + m1
        sc_ref[2 * b + 1:2 * b + 2, :] = (
            lax.rsqrt(var + np.float32(1e-5)) * gam_ref[...].astype(f32).reshape(1, D))

    def tail(ybuf, hbuf, ostage, osem):
        with jax.named_scope("inv"):
            for b in range(B):
                inverse(ybuf, hbuf, b)
        beta = bet_ref[...].astype(f32).reshape(1, D)
        CH = 32
        o32 = ostage.bitcast(jnp.uint32)

        def rows_out(r):
            ys = []
            for b in range(B):
                h = hbuf[b, pl.ds(r, CH), :].astype(f32)
                ys.append(_gelu((h - sc_ref[2 * b:2 * b + 1, :]) * sc_ref[2 * b + 1:2 * b + 2, :]
                                + beta))
            o32[pl.ds(r, CH), 0, :] = pltpu.pack_elementwise(ys, packed_dtype=bf16)

        def o_copy(r, n):
            return pltpu.make_async_copy(ostage.at[pl.ds(r, n)], o_hbm.at[pl.ds(r, n)],
                                         osem.at[0])

        def chunk(i, _):
            r = pl.multiple_of(i * OUT_ROWS, OUT_ROWS)

            def sub(t, _):
                rows_out(pl.multiple_of(r + t * CH, CH))
                return 0
            lax.fori_loop(0, OUT_ROWS // CH, sub, 0, unroll=2)
            o_copy(r, OUT_ROWS).start()
            return 0

        def wait(i, _):
            o_copy(pl.multiple_of(i * OUT_ROWS, OUT_ROWS), OUT_ROWS).wait()
            return 0

        nch = L // OUT_ROWS
        rem = L - nch * OUT_ROWS
        with jax.named_scope("finish"):
            lax.fori_loop(0, nch, chunk, 0)
            if rem:
                for t in range(-(-rem // CH)):
                    rows_out(nch * OUT_ROWS + t * CH)
                o_copy(nch * OUT_ROWS, rem).start()
            lax.fori_loop(0, nch, wait, 0)
            if rem:
                o_copy(nch * OUT_ROWS, rem).wait()

    dshape = pltpu.VMEM((CT, NF * MS, 128), jnp.uint32)

    def main(dlo):
        def front(wt_ref):
            with jax.named_scope("weights"):
                pl.run_scoped(functools.partial(weights, wt_ref),
                              pltpu.VMEM((K, D, D), bf16), pltpu.SemaphoreType.DMA((NWP,)))
            pl.run_scoped(functools.partial(fwd_mix, wt_ref, dlo), dshape)
        pl.run_scoped(front, pltpu.VMEM((NF, 2 * D, 2 * D), bf16))
        pl.run_scoped(functools.partial(tail, dlo),
                      pltpu.VMEM((B, HROWS, D), bf16), pltpu.VMEM((HROWS, B, D), bf16),
                      pltpu.SemaphoreType.DMA((1,)))
    pl.run_scoped(main, dshape)


@jax.jit
def pallas_standalone__self_sup_conv_stem_wavlm__speech_kernel(
    x: jax.Array,
    w: jax.Array,
    gn_gamma: jax.Array,
    gn_beta: jax.Array,
):
    B, T, D = x.shape
    K = w.shape[0]
    L = (T - K) // 2 + 1
    assert B == 2 and (K + 1) // 2 <= NTAP and D % 128 == 0 and T % 16 == 0
    NB = -(-L // M_OUT)
    NB = -(-NB // (2 * NSEG)) * (2 * NSEG)
    assert (B * NB) % 16 == 0
    hrows = NB * M_OUT
    xrows = max(2 * M_OUT * (NB - 1) + 2 * KP, T + 16)
    assert (NSEG - 1) * (NB // NSEG) * 2 * M_OUT < T <= NB * 2 * M_OUT
    f2, g8, a2 = _constants()
    dt = x.dtype
    consts = [jnp.asarray(c, dtype=jnp.bfloat16) for c in (f2, g8, a2)]

    vmem = pl.BlockSpec(memory_space=pltpu.VMEM)
    hbm = pl.BlockSpec(memory_space=pl.ANY)
    kern = functools.partial(_kernel, B=B, T=T, D=D, K=K, L=L, NB=NB, HROWS=hrows)
    out = pl.pallas_call(
        kern,
        in_specs=[hbm, hbm, vmem, vmem, vmem, vmem, vmem],
        out_specs=hbm,
        out_shape=jax.ShapeDtypeStruct((L, B, D), jnp.bfloat16),
        scratch_shapes=[
            pltpu.VMEM((xrows, D), bf16),
            pltpu.VMEM((8, D), f32),
            pltpu.SemaphoreType.DMA((NSEG,)),
        ],
        compiler_params=pltpu.CompilerParams(vmem_limit_bytes=127 * 1024 * 1024),
    )(x.astype(jnp.bfloat16), w.astype(jnp.bfloat16), gn_gamma, gn_beta, *consts)
    return jnp.transpose(out, (1, 0, 2)).astype(dt)
```
